```python
import os as _os
_os.environ.setdefault("JAX_PLATFORMS", "cpu")
import jax
import jax.numpy as jnp

def _softmax(x, axis=-1):
    return jax.nn.softmax(x, axis=axis)
def _gelu(x):
    return jax.nn.gelu(x, approximate=True)
def _silu(x):
    return jax.nn.silu(x)
def _sigmoid(x):
    return jax.nn.sigmoid(x)
def _layernorm(x, axis=-1, eps=1e-5):
    m = jnp.mean(x, axis=axis, keepdims=True)
    v = jnp.var(x, axis=axis, keepdims=True)
    return (x - m) / jnp.sqrt(v + eps)
def _scatter_add(tgt, idx, src, axis=0):
    return tgt.at[idx].add(src)
def _segment_sum(src, seg, n):
    return jax.ops.segment_sum(src, seg, n)
class _Rng:
    def __init__(self, key):
        self._k = key
    def _next(self):
        self._k, sub = jax.random.split(self._k)
        return sub
    def normal(self, shape):
        return jax.random.normal(self._next(), shape, dtype=jnp.bfloat16)
    def randint(self, lo, hi, shape):
        return jax.random.randint(self._next(), shape, lo, hi, dtype=jnp.int32)
    def uniform(self, shape, lo=0.0, hi=1.0):
        return jax.random.uniform(self._next(), shape, jnp.bfloat16, lo, hi)
    def permutation(self, n):
        return jax.random.permutation(self._next(), n)


kernel_name = 'gated_mix__mha_block__mha_block__prompt'

def setup_inputs():
    _rng = _Rng(jax.random.key(int.from_bytes(__import__("os").urandom(4), "little")))
    _w = (lambda a: (lambda t: t.astype(jnp.bfloat16) if jnp.issubdtype(t.dtype, jnp.floating) else t)(jnp.asarray(a)))
    def _A_setup():
        B, S, D, H = 1, 2048, 448, 16
        return {
            "x": _w((lambda *s: _rng.normal(s) * 0.05)(B, S, D)),
            "wqkv": _w((lambda *s: _rng.normal(s) * 0.4)(D, 3 * D)),
            "wo": _w((lambda *s: _rng.normal(s) * 0.05)(D, D)),
        }
    _A_in = _A_setup()

    def _B_setup():
        B, S, D, H = 1, 2048, 448, 16
        return {
            "x": _w((lambda *s: _rng.normal(s) * 0.05)(B, S, D)),
            "wqkv": _w((lambda *s: _rng.normal(s) * 0.4)(D, 3 * D)),
            "wo": _w((lambda *s: _rng.normal(s) * 0.05)(D, D)),
        }
    _B_in = _B_setup()

    return {
        "A_x": _A_in["x"],
        "A_wqkv": _A_in["wqkv"],
        "A_wo": _A_in["wo"],
        "B_x": _B_in["x"],
        "B_wqkv": _B_in["wqkv"],
        "B_wo": _B_in["wo"],
        "gate_w": _w((lambda *s: _rng.normal(s) * 0.05)(448) * 16.0),
    }

def reference(A_x, A_wqkv, A_wo, B_x, B_wqkv, B_wo, gate_w):
    def _A_ref(x, wqkv, wo):
        B, S, D = x.shape
        H = 16
        Dh = D // H
        qkv = (lambda x, *d: x.transpose(*d))((x @ wqkv).reshape(B, S, 3, H, Dh), 2, 0, 3, 1, 4)
        q, k, v = qkv[0], qkv[1], qkv[2]
        scores = jnp.einsum("bhqd,bhkd->bhqk", q, k) * (Dh ** -0.5)
        p = _softmax(scores, axis=-1)
        o = jnp.einsum("bhqk,bhkd->bhqd", p, v)
        return (lambda x, *d: x.transpose(*d))(o, 0, 2, 1, 3).reshape(B, S, D) @ wo

    def _B_ref(x, wqkv, wo):
        B, S, D = x.shape
        H = 16
        Dh = D // H
        qkv = (lambda x, *d: x.transpose(*d))((x @ wqkv).reshape(B, S, 3, H, Dh), 2, 0, 3, 1, 4)
        q, k, v = qkv[0], qkv[1], qkv[2]
        scores = jnp.einsum("bhqd,bhkd->bhqk", q, k) * (Dh ** -0.5)
        p = _softmax(scores, axis=-1)
        o = jnp.einsum("bhqk,bhkd->bhqd", p, v)
        return (lambda x, *d: x.transpose(*d))(o, 0, 2, 1, 3).reshape(B, S, D) @ wo

    x = A_x
    g = _sigmoid((x * gate_w).sum(-1, keepdims=True))
    a = _A_ref(x, A_wqkv, A_wo)
    b = _B_ref(x, B_wqkv, B_wo)
    return g * a + (1 - g) * b
```

```python
import math

import jax
import jax.numpy as jnp
from jax import lax
import jax.experimental.pallas as pl
import jax.experimental.pallas.tpu as pltpu

S, D, H, DH, DP = 2048, 448, 16, 28, 32
NT = (((1,), (1,)), ((), ()))
TQ = 512


def _kernel(x_ref, xq_ref, wT_ref, woT_ref, gate_ref, o_ref, k_scr, vT_scr, qT_scr, oT_scr):
    tq = TQ
    i = pl.program_id(0)

    @pl.when(i == 0)
    def _():
        x = x_ref[...]
        for m in range(2):
            k = lax.dot_general(x, wT_ref[m, 1], NT, preferred_element_type=jnp.float32)
            for g in range(4):
                k_scr[m * 4 + g] = k[:, g * 128:(g + 1) * 128].astype(jnp.bfloat16)
            vT = lax.dot_general(wT_ref[m, 2], x, NT, preferred_element_type=jnp.float32)
            row = lax.broadcasted_iota(jnp.int32, vT.shape, 0)
            vT = jnp.where(row % DP == DH, 1.0, vT)
            vT_scr[pl.ds(m * 16, 16)] = vT.astype(jnp.bfloat16).reshape(16, DP, S)

    xq = xq_ref[...]
    c = (DH ** -0.5) * math.log2(math.e)
    for m in range(2):
        qT = lax.dot_general(wT_ref[m, 0], xq, NT, preferred_element_type=jnp.float32)
        qT_scr[pl.ds(m * 4, 4)] = (qT * c).astype(jnp.bfloat16).reshape(4, 128, tq)
    gl = lax.dot_general(gate_ref[...], xq, NT, preferred_element_type=jnp.float32)[0:1]
    g = jax.nn.sigmoid(gl)

    def body(hh, carry):
        grp = hh // 4
        j = hh % 4
        kg = k_scr[grp]
        qg = qT_scr[grp]
        row = lax.broadcasted_iota(jnp.int32, qg.shape, 0)
        qz = jnp.where(row // DP == j, qg, jnp.zeros_like(qg))
        sT = jnp.dot(kg, qz, preferred_element_type=jnp.float32)
        mx = jnp.max(sT, axis=0, keepdims=True)
        p = jnp.exp2(sT - mx).astype(jnp.bfloat16)
        oT = jnp.dot(vT_scr[hh], p, preferred_element_type=jnp.float32)
        l = oT[DH:DH + 1]
        gg = jnp.where(hh < 16, g, 1.0 - g)
        oT = oT * (gg / l)
        oT_scr[pl.ds(pl.multiple_of(hh * DP, DP), DP), :] = oT.astype(jnp.bfloat16)
        return carry

    lax.fori_loop(0, 32, body, 0)
    outT = jnp.dot(woT_ref[...], oT_scr[...], preferred_element_type=jnp.float32)
    o_ref[...] = outT.T.astype(o_ref.dtype)


@jax.jit
def pallas_gated_mix__mha_block__mha_block__prompt_kernel(
    A_x: jax.Array,
    A_wqkv: jax.Array,
    A_wo: jax.Array,
    B_x: jax.Array,
    B_wqkv: jax.Array,
    B_wo: jax.Array,
    gate_w: jax.Array,
):
    tq = TQ
    x = A_x.reshape(S, D)
    w = jnp.stack([A_wqkv, B_wqkv]).reshape(2, D, 3, H, DH)
    w = jnp.pad(w, ((0, 0), (0, 0), (0, 0), (0, 0), (0, DP - DH)))
    wT = w.reshape(2, D, 3, H * DP).transpose(0, 2, 3, 1)
    wo = jnp.stack([A_wo, B_wo]).reshape(2, H, DH, D)
    wo = jnp.pad(wo, ((0, 0), (0, 0), (0, DP - DH), (0, 0))).reshape(2 * H * DP, D)
    woT = wo.T
    gate = jnp.pad(gate_w.reshape(1, D), ((0, 15), (0, 0)))
    out = pl.pallas_call(
        _kernel,
        grid=(S // tq,),
        in_specs=[
            pl.BlockSpec((S, D), lambda i: (0, 0)),
            pl.BlockSpec((tq, D), lambda i: (i, 0)),
            pl.BlockSpec((2, 3, 512, D), lambda i: (0, 0, 0, 0)),
            pl.BlockSpec((D, 1024), lambda i: (0, 0)),
            pl.BlockSpec((16, D), lambda i: (0, 0)),
        ],
        out_specs=pl.BlockSpec((tq, D), lambda i: (i, 0)),
        out_shape=jax.ShapeDtypeStruct((S, D), jnp.bfloat16),
        scratch_shapes=[
            pltpu.VMEM((8, S, 128), jnp.bfloat16),
            pltpu.VMEM((32, DP, S), jnp.bfloat16),
            pltpu.VMEM((8, 128, tq), jnp.bfloat16),
            pltpu.VMEM((1024, tq), jnp.bfloat16),
        ],
        compiler_params=pltpu.CompilerParams(
            dimension_semantics=("arbitrary",), vmem_limit_bytes=100 * 2**20),
    )(x, x, wT, woT, gate)
    return out.reshape(1, S, D)
```

```python
import math

import jax
import jax.numpy as jnp
from jax import lax
import jax.experimental.pallas as pl
import jax.experimental.pallas.tpu as pltpu

S, D, H, DH, DP = 2048, 448, 16, 28, 32
WSTART = (0, 112, 224, 320)
TQ = 512
KC = 128
U = 4
NC = S // KC
NT = S // TQ
NSTEP = NT * 2 * H
NPC = TQ // 128


def _kernel(xT_hbm, wA_hbm, wB_hbm, woA_hbm, woB_hbm, gate_hbm, o_hbm,
            xT_ref, wA_ref, wB_ref, woA_ref, woB_ref, gate_ref, o_ref, sems, osems,
            k_scr, vT_scr, qT_scr, oT_scr, g_scr, wo_scr, *bufs):
    tq, kc = TQ, KC
    cp_wA = pltpu.make_async_copy(wA_hbm, wA_ref, sems.at[0])
    cp_x = [pltpu.make_async_copy(xT_hbm.at[:, pl.ds(t * tq, tq)], xT_ref.at[:, pl.ds(t * tq, tq)],
                                  sems.at[1 + t]) for t in range(NT)]
    cp_rest = [pltpu.make_async_copy(s, d, sems.at[1 + NT + i]) for i, (s, d) in enumerate(
        ((wB_hbm, wB_ref), (woA_hbm, woA_ref), (woB_hbm, woB_ref), (gate_hbm, gate_ref)))]
    cp_wA.start()
    cp_x[0].start()

    c = (DH ** -0.5) * math.log2(math.e)
    zpad = jnp.zeros((DP - DH, D), jnp.bfloat16)

    def pad_heads(w):
        return jnp.concatenate(
            [piece for h in range(H) for piece in (w[DH * h:DH * (h + 1)], zpad)], axis=0)

    def prep_w(w_ref):
        wT = w_ref[...].T
        return wT[0:D], wT[D:2 * D], pad_heads(wT[2 * D:3 * D])

    def proj(m, ws, t_lo, t_hi):
        wq, wk, wvp = ws
        cols = pl.ds(t_lo * tq, (t_hi - t_lo) * tq)
        xc = xT_ref[:, cols]
        qT = jnp.dot(wq, xc, preferred_element_type=jnp.float32)
        qT = (qT * c).astype(jnp.bfloat16)
        for t in range(t_lo, t_hi):
            for w in range(4):
                qT_scr[t, m * 4 + w] = qT[WSTART[w]:WSTART[w] + 128,
                                          (t - t_lo) * tq:(t - t_lo + 1) * tq]
        kT = jnp.dot(wk, xc, preferred_element_type=jnp.float32)
        for w in range(4):
            k_scr[m * 4 + w, cols, :] = kT[WSTART[w]:WSTART[w] + 128].T.astype(jnp.bfloat16)
        vT = jnp.dot(wvp, xc, preferred_element_type=jnp.float32)
        row = lax.broadcasted_iota(jnp.int32, vT.shape, 0)
        vT = jnp.where(row % DP == DH, 1.0, vT)
        vT_scr[pl.ds(m * H, H), :, cols] = vT.astype(jnp.bfloat16).reshape(H, DP, vT.shape[1])

    cp_wA.wait()
    cp_x[0].wait()
    for cp in cp_x[1:]:
        cp.start()
    for cp in cp_rest:
        cp.start()
    wsA = prep_w(wA_ref)
    proj(0, wsA, 0, 1)
    for cp in cp_x[1:]:
        cp.wait()
    proj(0, wsA, 1, NT)
    for cp in cp_rest:
        cp.wait()
    wsB = prep_w(wB_ref)
    proj(1, wsB, 0, NT)
    for m, wo_ref in enumerate((woA_ref, woB_ref)):
        wo_scr[:, pl.ds(m * H * DP, H * DP)] = pad_heads(wo_ref[...]).T
    gl = jnp.dot(gate_ref[...], xT_ref[...], preferred_element_type=jnp.float32)[0:8]
    gfull = jax.nn.sigmoid(gl)
    for t in range(NT):
        g_scr[t] = gfull[:, t * tq:(t + 1) * tq]

    def step(n2, n0, sb, m0, extra=None):
        if n2 is not None:
            t2 = n2 // (2 * H)
            h2 = n2 % (2 * H)
            grp = h2 // 4
            off = (h2 % 4) * DH + jnp.where(grp % 4 == 3, 16, 0)
            qg = qT_scr[t2, grp]
            row = lax.broadcasted_iota(jnp.int32, qg.shape, 0)
            qz = jnp.where((row >= off) & (row < off + DH), qg, jnp.zeros_like(qg))
        if n0 is not None:
            t0 = n0 // (2 * H)
            h0 = n0 % (2 * H)
        mp = None
        acc = None
        for cidx in range(NC):
            sl = pl.ds(cidx * kc, kc)
            if n0 is not None:
                p = jnp.exp2(sb[sl, :] - m0).astype(jnp.bfloat16)
                o = jnp.dot(vT_scr[h0, :, sl], p, preferred_element_type=jnp.float32)
                acc = o if acc is None else acc + o
            if n2 is not None:
                sT = jnp.dot(k_scr[grp, sl, :], qz, preferred_element_type=jnp.float32)
                sb[sl, :] = sT
                mc = jnp.max(sT.reshape(kc // 8, 8, tq), axis=0)
                mp = mc if mp is None else jnp.maximum(mp, mc)
            if extra is not None:
                extra(cidx)
        if n0 is not None:
            l = acc[DH:DH + 1]
            g = g_scr[t0, 0:1, :]
            gg = jnp.where(h0 < H, g, 1.0 - g)
            oT = acc * (gg / l)
            oT_scr[t0, pl.ds(pl.multiple_of(h0 * DP, DP), DP), :] = oT.astype(jnp.bfloat16)
        if n2 is not None:
            return jnp.max(mp, axis=0, keepdims=True)

    def ocopy(t, j):
        cs = pl.ds(t * tq + j * 128, 128)
        return pltpu.make_async_copy(o_ref.at[:, cs], o_hbm.at[:, cs], osems.at[t * NPC + j])

    def outproj(t, j):
        o_ref[:, pl.ds(t * tq + j * 128, 128)] = jnp.dot(
            wo_scr[...], oT_scr[t, :, pl.ds(j * 128, 128)],
            preferred_element_type=jnp.float32).astype(o_ref.dtype)
        ocopy(t, j).start()

    ms = tuple(step(u, None, bufs[u], None) for u in range(U))

    def body(t, ms):
        return tuple(step(U * t + u + U, U * t + u, bufs[u], ms[u]) for u in range(U))

    ms = lax.fori_loop(0, NSTEP // U - 1, body, ms)

    pieces = [(t, j) for t in range(NT - 1) for j in range(NPC)]
    slots = U * NC
    sched = {}
    for pi, pc in enumerate(pieces):
        sched.setdefault((pi * slots) // len(pieces), []).append(pc)
    for u in range(U):
        def extra(cidx, u=u):
            for pc in sched.get(u * NC + cidx, []):
                outproj(*pc)
        step(None, NSTEP - U + u, bufs[u], ms[u], extra)
    for j in range(NPC):
        outproj(NT - 1, j)
    for t in range(NT):
        for j in range(NPC):
            ocopy(t, j).wait()


@jax.jit
def pallas_gated_mix__mha_block__mha_block__prompt_kernel(
    A_x: jax.Array,
    A_wqkv: jax.Array,
    A_wo: jax.Array,
    B_x: jax.Array,
    B_wqkv: jax.Array,
    B_wo: jax.Array,
    gate_w: jax.Array,
):
    bf = jnp.bfloat16
    xT = A_x.reshape(S, D).T
    gate = jnp.pad(gate_w.reshape(1, D), ((0, 15), (0, 0)))
    outT = pl.pallas_call(
        _kernel,
        in_specs=[pl.BlockSpec(memory_space=pl.ANY)] * 6,
        out_specs=pl.BlockSpec(memory_space=pl.ANY),
        out_shape=jax.ShapeDtypeStruct((D, S), bf),
        scratch_shapes=[
            pltpu.VMEM((D, S), bf), pltpu.VMEM((D, 3 * D), bf), pltpu.VMEM((D, 3 * D), bf),
            pltpu.VMEM((D, D), bf), pltpu.VMEM((D, D), bf), pltpu.VMEM((16, D), bf),
            pltpu.VMEM((D, S), bf),
            pltpu.SemaphoreType.DMA((5 + NT,)), pltpu.SemaphoreType.DMA((S // 128,)),
            pltpu.VMEM((8, S, 128), bf),
            pltpu.VMEM((2 * H, DP, S), bf),
            pltpu.VMEM((NT, 8, 128, TQ), bf),
            pltpu.VMEM((NT, 2 * H * DP, TQ), bf),
            pltpu.VMEM((NT, 8, TQ), jnp.float32),
            pltpu.VMEM((D, 2 * H * DP), bf),
        ] + [pltpu.VMEM((S, TQ), jnp.float32)] * U,
        compiler_params=pltpu.CompilerParams(vmem_limit_bytes=100 * 2**20),
    )(xT, A_wqkv, B_wqkv, A_wo, B_wo, gate)
    return outT.T.reshape(1, S, D)
```

```python
import math

import jax
import jax.numpy as jnp
from jax import lax
import jax.experimental.pallas as pl
import jax.experimental.pallas.tpu as pltpu

S, D, H, DH, DP = 2048, 448, 16, 28, 32
WSTART = (0, 112, 224, 320)
TQ = 512
KC = 128
U = 4
NC = S // KC
NT = S // TQ
NSTEP = NT * 2 * H
NPC = TQ // 128
WSPLIT = 512


def _kernel(xT_hbm, wA_hbm, wB_hbm, woA_hbm, woB_hbm, gate_hbm, o_hbm,
            xT_ref, wA_ref, wB_ref, wo_scr, gate_ref, o_ref, sems, osems,
            k_scr, vT_scr, qT_scr, oT_scr, g_scr, *bufs):
    tq, kc = TQ, KC
    f32, bf16 = jnp.float32, jnp.bfloat16

    cp_first = pltpu.make_async_copy(
        wA_hbm.at[:, pl.ds(0, WSPLIT)], wA_ref.at[:, pl.ds(0, WSPLIT)], sems.at[0])
    cp_second = [
        pltpu.make_async_copy(wA_hbm.at[:, pl.ds(WSPLIT, 3 * D - WSPLIT)],
                              wA_ref.at[:, pl.ds(WSPLIT, 3 * D - WSPLIT)], sems.at[1]),
        pltpu.make_async_copy(gate_hbm, gate_ref, sems.at[2])]
    cp_rest = [pltpu.make_async_copy(s, d, sems.at[3 + i]) for i, (s, d) in enumerate(
        ((wB_hbm, wB_ref), (woA_hbm, wo_scr.at[pl.ds(0, D)]), (woB_hbm, wo_scr.at[pl.ds(D, D)])))]
    cp_x = [pltpu.make_async_copy(xT_hbm.at[:, pl.ds(t * tq, tq)], xT_ref.at[:, pl.ds(t * tq, tq)],
                                  sems.at[6 + t]) for t in range(NT)]
    cp_first.start()
    cp_x[0].start()
    for cp in cp_second:
        cp.start()

    c = (DH ** -0.5) * math.log2(math.e)

    def prep_w(w_ref, gate_row=None):
        wT = w_ref[...].T
        wv = wT[2 * D:3 * D]
        if gate_row is not None:
            wv = jnp.concatenate([wv, gate_row, jnp.zeros((15, D), bf16)], axis=0)
        return wT[0:D], wT[D:2 * D], wv

    def projq(m, wq, t_lo, t_hi):
        xc = xT_ref[:, pl.ds(t_lo * tq, (t_hi - t_lo) * tq)]
        qT = jnp.dot(wq, xc, preferred_element_type=f32)
        qT = (qT * c).astype(bf16)
        for t in range(t_lo, t_hi):
            for w in range(4):
                qT_scr[t, m * 4 + w] = qT[WSTART[w]:WSTART[w] + 128,
                                          (t - t_lo) * tq:(t - t_lo + 1) * tq]

    def proj(m, ws, t_lo, t_hi, doq=True):
        wq, wk, wv = ws
        if doq:
            projq(m, wq, t_lo, t_hi)
        cols = pl.ds(t_lo * tq, (t_hi - t_lo) * tq)
        xc = xT_ref[:, cols]
        kT = jnp.dot(wk, xc, preferred_element_type=f32)
        for w in range(4):
            k_scr[m * 4 + w, cols, :] = kT[WSTART[w]:WSTART[w] + 128].T.astype(bf16)
        vT = jnp.dot(wv, xc, preferred_element_type=f32)
        ncols = vT.shape[1]
        if m == 0:
            g = jax.nn.sigmoid(vT[D:D + 8])
            for t in range(t_lo, t_hi):
                g_scr[t] = g[:, (t - t_lo) * tq:(t - t_lo + 1) * tq]
        tail = jnp.concatenate(
            [jnp.ones((1, ncols), f32), jnp.zeros((DP - DH - 1, ncols), f32)], axis=0)
        for h in range(H):
            blk = jnp.concatenate([vT[DH * h:DH * (h + 1)], tail], axis=0)
            vT_scr[m * H + h, :, cols] = blk.astype(bf16)

    cp_first.wait()
    cp_x[0].wait()
    projq(0, wA_ref[:, 0:WSPLIT].T[0:D], 0, 1)
    for cp in cp_second:
        cp.wait()
    for cp in cp_x[1:]:
        cp.start()
    for cp in cp_rest:
        cp.start()
    wsA = prep_w(wA_ref, gate_ref[...].reshape(1, D))
    proj(0, wsA, 0, 1, doq=False)
    for cp in cp_x[1:]:
        cp.wait()
    proj(0, wsA, 1, NT)
    for cp in cp_rest:
        cp.wait()
    proj(1, prep_w(wB_ref), 0, NT)

    def step(n2, n0, sb, m0, extra=None):
        if n2 is not None:
            t2 = n2 // (2 * H)
            h2 = n2 % (2 * H)
            grp = h2 // 4
            off = (h2 % 4) * DH + jnp.where(grp % 4 == 3, 16, 0)
            qg = qT_scr[t2, grp]
            row = lax.broadcasted_iota(jnp.int32, qg.shape, 0)
            qz = jnp.where((row >= off) & (row < off + DH), qg, jnp.zeros_like(qg))
        if n0 is not None:
            t0 = n0 // (2 * H)
            h0 = n0 % (2 * H)
        mp = None
        acc = None
        for cidx in range(NC):
            sl = pl.ds(cidx * kc, kc)
            if n0 is not None:
                p = jnp.exp2(sb[sl, :] - m0).astype(bf16)
                o = jnp.dot(vT_scr[h0, :, sl], p, preferred_element_type=f32)
                acc = o if acc is None else acc + o
            if n2 is not None:
                sT = jnp.dot(k_scr[grp, sl, :], qz, preferred_element_type=f32)
                sb[sl, :] = sT
                mc = jnp.max(sT.reshape(kc // 8, 8, tq), axis=0)
                mp = mc if mp is None else jnp.maximum(mp, mc)
            if extra is not None:
                extra(cidx)
        if n0 is not None:
            l = acc[DH:DH + 1]
            g = g_scr[t0, 0:1, :]
            gg = jnp.where(h0 < H, g, 1.0 - g)
            oT = acc * (gg / l)
            oT_scr[t0, pl.ds(pl.multiple_of(h0 * DP, DP), DP), :] = oT.astype(bf16)
        if n2 is not None:
            return jnp.max(mp, axis=0, keepdims=True)

    ms = tuple(step(u, None, bufs[u], None) for u in range(U))

    def body(t, ms):
        return tuple(step(U * t + u + U, U * t + u, bufs[u], ms[u]) for u in range(U))

    ms = lax.fori_loop(0, NSTEP // U - 1, body, ms)

    woT = wo_scr[...].T

    def ocopy(t, j):
        cs = pl.ds(t * tq + j * 128, 128)
        return pltpu.make_async_copy(o_ref.at[:, cs], o_hbm.at[:, cs], osems.at[t * NPC + j])

    def outproj(t, j):
        op = oT_scr[t, :, pl.ds(j * 128, 128)]
        oc = jnp.concatenate([op[DP * h:DP * h + DH] for h in range(2 * H)], axis=0)
        o_ref[:, pl.ds(t * tq + j * 128, 128)] = jnp.dot(
            woT, oc, preferred_element_type=f32).astype(o_ref.dtype)
        ocopy(t, j).start()

    pieces = [(t, j) for t in range(NT - 1) for j in range(NPC)]
    slots = U * NC
    sched = {}
    for pi, pc in enumerate(pieces):
        sched.setdefault((pi * slots) // len(pieces), []).append(pc)
    for u in range(U):
        def extra(cidx, u=u):
            for pc in sched.get(u * NC + cidx, []):
                outproj(*pc)
        step(None, NSTEP - U + u, bufs[u], ms[u], extra)
    for j in range(NPC):
        outproj(NT - 1, j)
    for t in range(NT):
        for j in range(NPC):
            ocopy(t, j).wait()


@jax.jit
def pallas_gated_mix__mha_block__mha_block__prompt_kernel(
    A_x: jax.Array,
    A_wqkv: jax.Array,
    A_wo: jax.Array,
    B_x: jax.Array,
    B_wqkv: jax.Array,
    B_wo: jax.Array,
    gate_w: jax.Array,
):
    bf = jnp.bfloat16
    xT = A_x.reshape(S, D).T
    outT = pl.pallas_call(
        _kernel,
        in_specs=[pl.BlockSpec(memory_space=pl.ANY)] * 6,
        out_specs=pl.BlockSpec(memory_space=pl.ANY),
        out_shape=jax.ShapeDtypeStruct((D, S), bf),
        scratch_shapes=[
            pltpu.VMEM((D, S), bf), pltpu.VMEM((D, 3 * D), bf), pltpu.VMEM((D, 3 * D), bf),
            pltpu.VMEM((2 * D, D), bf), pltpu.VMEM((D,), bf), pltpu.VMEM((D, S), bf),
            pltpu.SemaphoreType.DMA((6 + NT,)), pltpu.SemaphoreType.DMA((S // 128,)),
            pltpu.VMEM((8, S, 128), bf),
            pltpu.VMEM((2 * H, DP, S), bf),
            pltpu.VMEM((NT, 8, 128, TQ), bf),
            pltpu.VMEM((NT, 2 * H * DP, TQ), bf),
            pltpu.VMEM((NT, 8, TQ), jnp.float32),
        ] + [pltpu.VMEM((S, TQ), jnp.float32)] * U,
        compiler_params=pltpu.CompilerParams(vmem_limit_bytes=100 * 2**20),
    )(xT, A_wqkv, B_wqkv, A_wo, B_wo, gate_w)
    return outT.T.reshape(1, S, D)
```

```python
import math

import jax
import jax.numpy as jnp
from jax import lax
import jax.experimental.pallas as pl
import jax.experimental.pallas.tpu as pltpu

S, D, H, DH, DP = 2048, 448, 16, 28, 32
WSTART = (0, 112, 224, 320)
TQ = 512
KC = 128
U = 4
LAG = 1
NC = S // KC
NT = S // TQ
NSTEP = NT * 2 * H
NPC = TQ // 128
WSPLIT = 512


def _kernel(xT_hbm, wA_hbm, wB_hbm, woA_hbm, woB_hbm, gate_hbm, o_hbm,
            xT_ref, wA_ref, wB_ref, wo_scr, gate_ref, o_ref, sems, osems,
            k_scr, vT_scr, qT_scr, oT_scr, g_scr, *bufs):
    tq, kc = TQ, KC
    f32, bf16 = jnp.float32, jnp.bfloat16

    cp_first = pltpu.make_async_copy(
        wA_hbm.at[:, pl.ds(0, WSPLIT)], wA_ref.at[:, pl.ds(0, WSPLIT)], sems.at[0])
    cp_second = [
        pltpu.make_async_copy(wA_hbm.at[:, pl.ds(WSPLIT, 3 * D - WSPLIT)],
                              wA_ref.at[:, pl.ds(WSPLIT, 3 * D - WSPLIT)], sems.at[1]),
        pltpu.make_async_copy(gate_hbm, gate_ref, sems.at[2])]
    cp_rest = [pltpu.make_async_copy(s, d, sems.at[3 + i]) for i, (s, d) in enumerate(
        ((wB_hbm, wB_ref), (woA_hbm, wo_scr.at[pl.ds(0, D)]), (woB_hbm, wo_scr.at[pl.ds(D, D)])))]
    cp_x = [pltpu.make_async_copy(xT_hbm.at[:, pl.ds(t * tq, tq)], xT_ref.at[:, pl.ds(t * tq, tq)],
                                  sems.at[6 + t]) for t in range(NT)]
    cp_first.start()
    cp_x[0].start()
    for cp in cp_second:
        cp.start()

    c = (DH ** -0.5) * math.log2(math.e)

    def prep_w(w_ref, gate_row=None):
        wT = w_ref[...].T
        wv = wT[2 * D:3 * D]
        if gate_row is not None:
            wv = jnp.concatenate([wv, gate_row, jnp.zeros((15, D), bf16)], axis=0)
        return wT[0:D], wT[D:2 * D], wv

    def projq(m, wq, t_lo, t_hi):
        xc = xT_ref[:, pl.ds(t_lo * tq, (t_hi - t_lo) * tq)]
        qT = jnp.dot(wq, xc, preferred_element_type=f32)
        qT = (qT * c).astype(bf16)
        for t in range(t_lo, t_hi):
            for w in range(4):
                qT_scr[t, m * 4 + w] = qT[WSTART[w]:WSTART[w] + 128,
                                          (t - t_lo) * tq:(t - t_lo + 1) * tq]

    def proj(m, ws, t_lo, t_hi, doq=True):
        wq, wk, wv = ws
        if doq:
            projq(m, wq, t_lo, t_hi)
        cols = pl.ds(t_lo * tq, (t_hi - t_lo) * tq)
        xc = xT_ref[:, cols]
        kT = jnp.dot(wk, xc, preferred_element_type=f32)
        for w in range(4):
            k_scr[m * 4 + w, cols, :] = kT[WSTART[w]:WSTART[w] + 128].T.astype(bf16)
        vT = jnp.dot(wv, xc, preferred_element_type=f32)
        ncols = vT.shape[1]
        if m == 0:
            g = jax.nn.sigmoid(vT[D:D + 8])
            for t in range(t_lo, t_hi):
                g_scr[t] = g[:, (t - t_lo) * tq:(t - t_lo + 1) * tq]
        tail = jnp.concatenate(
            [jnp.ones((1, ncols), f32), jnp.zeros((DP - DH - 1, ncols), f32)], axis=0)
        for h in range(H):
            blk = jnp.concatenate([vT[DH * h:DH * (h + 1)], tail], axis=0)
            vT_scr[m * H + h, :, cols] = blk.astype(bf16)

    cp_first.wait()
    cp_x[0].wait()
    projq(0, wA_ref[:, 0:WSPLIT].T[0:D], 0, 1)
    for cp in cp_second:
        cp.wait()
    for cp in cp_x[1:]:
        cp.start()
    for cp in cp_rest:
        cp.start()
    wsA = prep_w(wA_ref, gate_ref[...].reshape(1, D))
    proj(0, wsA, 0, 1, doq=False)
    for cp in cp_x[1:]:
        cp.wait()
    proj(0, wsA, 1, NT)
    for cp in cp_rest:
        cp.wait()
    proj(1, prep_w(wB_ref), 0, NT)

    def step(n2, n0, sb, m0, extra=None):
        if n2 is not None:
            t2 = n2 // (2 * H)
            h2 = n2 % (2 * H)
            grp = h2 // 4
            off = (h2 % 4) * DH + jnp.where(grp % 4 == 3, 16, 0)
            qg = qT_scr[t2, grp]
            row = lax.broadcasted_iota(jnp.int32, qg.shape, 0)
            qz = jnp.where((row >= off) & (row < off + DH), qg, jnp.zeros_like(qg))
        if n0 is not None:
            t0 = n0 // (2 * H)
            h0 = n0 % (2 * H)
            m0 = jnp.max(m0, axis=0, keepdims=True)
        mp = None
        acc = None
        for cidx in range(NC + LAG):
            if n0 is not None and cidx < NC:
                sl = pl.ds(cidx * kc, kc)
                p = jnp.exp2(sb[sl, :] - m0).astype(bf16)
                o = jnp.dot(vT_scr[h0, :, sl], p, preferred_element_type=f32)
                acc = o if acc is None else acc + o
            if n2 is not None and cidx >= LAG:
                sl2 = pl.ds((cidx - LAG) * kc, kc)
                sT = jnp.dot(k_scr[grp, sl2, :], qz, preferred_element_type=f32)
                sb[sl2, :] = sT
                mc = jnp.max(sT.reshape(kc // 8, 8, tq), axis=0)
                mp = mc if mp is None else jnp.maximum(mp, mc)
            if extra is not None and cidx < NC:
                extra(cidx)
        if n0 is not None:
            l = acc[DH:DH + 1]
            g = g_scr[t0, 0:1, :]
            gg = jnp.where(h0 < H, g, 1.0 - g)
            oT = acc * (gg / l)
            oT_scr[t0, pl.ds(pl.multiple_of(h0 * DP, DP), DP), :] = oT.astype(bf16)
        if n2 is not None:
            return mp

    ms = tuple(step(u, None, bufs[u], None) for u in range(U))

    def body(t, ms):
        return tuple(step(U * t + u + U, U * t + u, bufs[u], ms[u]) for u in range(U))

    ms = lax.fori_loop(0, NSTEP // U - 1, body, ms)

    woT = wo_scr[...].T

    def ocopy(t, j):
        cs = pl.ds(t * tq + j * 128, 128)
        return pltpu.make_async_copy(o_ref.at[:, cs], o_hbm.at[:, cs], osems.at[t * NPC + j])

    def outproj(t, j):
        op = oT_scr[t, :, pl.ds(j * 128, 128)]
        oc = jnp.concatenate([op[DP * h:DP * h + DH] for h in range(2 * H)], axis=0)
        o_ref[:, pl.ds(t * tq + j * 128, 128)] = jnp.dot(
            woT, oc, preferred_element_type=f32).astype(o_ref.dtype)
        ocopy(t, j).start()

    pieces = [(t, j) for t in range(NT - 1) for j in range(NPC)]
    slots = U * NC
    sched = {}
    for pi, pc in enumerate(pieces):
        sched.setdefault((pi * slots) // len(pieces), []).append(pc)
    for u in range(U):
        def extra(cidx, u=u):
            for pc in sched.get(u * NC + cidx, []):
                outproj(*pc)
        step(None, NSTEP - U + u, bufs[u], ms[u], extra)
    for j in range(NPC):
        outproj(NT - 1, j)
    for t in range(NT):
        for j in range(NPC):
            ocopy(t, j).wait()


@jax.jit
def pallas_gated_mix__mha_block__mha_block__prompt_kernel(
    A_x: jax.Array,
    A_wqkv: jax.Array,
    A_wo: jax.Array,
    B_x: jax.Array,
    B_wqkv: jax.Array,
    B_wo: jax.Array,
    gate_w: jax.Array,
):
    bf = jnp.bfloat16
    xT = A_x.reshape(S, D).T
    outT = pl.pallas_call(
        _kernel,
        in_specs=[pl.BlockSpec(memory_space=pl.ANY)] * 6,
        out_specs=pl.BlockSpec(memory_space=pl.ANY),
        out_shape=jax.ShapeDtypeStruct((D, S), bf),
        scratch_shapes=[
            pltpu.VMEM((D, S), bf), pltpu.VMEM((D, 3 * D), bf), pltpu.VMEM((D, 3 * D), bf),
            pltpu.VMEM((2 * D, D), bf), pltpu.VMEM((D,), bf), pltpu.VMEM((D, S), bf),
            pltpu.SemaphoreType.DMA((6 + NT,)), pltpu.SemaphoreType.DMA((S // 128,)),
            pltpu.VMEM((8, S, 128), bf),
            pltpu.VMEM((2 * H, DP, S), bf),
            pltpu.VMEM((NT, 8, 128, TQ), bf),
            pltpu.VMEM((NT, 2 * H * DP, TQ), bf),
            pltpu.VMEM((NT, 8, TQ), jnp.float32),
        ] + [pltpu.VMEM((S, TQ), jnp.float32)] * U,
        compiler_params=pltpu.CompilerParams(vmem_limit_bytes=100 * 2**20),
    )(xT, A_wqkv, B_wqkv, A_wo, B_wo, gate_w)
    return outT.T.reshape(1, S, D)
```
